```python
import os as _os
_os.environ.setdefault('JAX_PLATFORMS', 'cpu')
import jax
import jax.numpy as jnp

def _softmax(x, axis=-1):
    return jax.nn.softmax(x, axis=axis)

def _gelu(x):
    return jax.nn.gelu(x, approximate=True)

def _silu(x):
    return jax.nn.silu(x)

def _sigmoid(x):
    return jax.nn.sigmoid(x)

def _layernorm(x, axis=-1, eps=1e-05):
    m = jnp.mean(x, axis=axis, keepdims=True)
    v = jnp.var(x, axis=axis, keepdims=True)
    return (x - m) / jnp.sqrt(v + eps)

def _scatter_add(tgt, idx, src, axis=0):
    return tgt.at[idx].add(src)

def _segment_sum(src, seg, n):
    return jax.ops.segment_sum(src, seg, n)

class _Rng:

    def __init__(self, key):
        self._k = key

    def _next(self):
        self._k, sub = jax.random.split(self._k)
        return sub

    def normal(self, shape):
        return jax.random.normal(self._next(), shape, dtype=jnp.bfloat16)

    def randint(self, lo, hi, shape):
        return jax.random.randint(self._next(), shape, lo, hi, dtype=jnp.int32)

    def uniform(self, shape, lo=0.0, hi=1.0):
        return jax.random.uniform(self._next(), shape, jnp.bfloat16, lo, hi)

    def permutation(self, n):
        return jax.random.permutation(self._next(), n)
kernel_name = 'adaLN_cond__sliding_local_dilated__dense_activation_relu__prompt'

def setup_inputs():
    _rng = _Rng(jax.random.key(int.from_bytes(__import__("os").urandom(4), "little")))
    _w = lambda a: (lambda t: t.astype(jnp.bfloat16) if jnp.issubdtype(t.dtype, jnp.floating) else t)(jnp.asarray(a))

    def _A_setup():
        B, S, D = (1, 2048, 576)
        return {'x': _w((lambda *s: _rng.normal(s) * 0.05)(B, S, D)), 'wqkv': _w((lambda *s: _rng.normal(s) * 0.05)(D, 3 * D)), 'wo': _w((lambda *s: _rng.normal(s) * 0.05)(D, D))}
    _A_in = _A_setup()

    def _B_setup():
        B, S, D, Dff = (1, 2048, 576, 4608)
        return {'x': _w((lambda *s: _rng.normal(s) * 0.05)(B, S, D)), 'w1': _w((lambda *s: _rng.normal(s) * 0.05)(D, Dff)), 'w2': _w((lambda *s: _rng.normal(s) * 0.05)(Dff, D))}
    _B_in = _B_setup()
    return {'A_x': _A_in['x'], 'A_wqkv': _A_in['wqkv'], 'A_wo': _A_in['wo'], 'B_x': _B_in['x'], 'B_w1': _B_in['w1'], 'B_w2': _B_in['w2'], 'c': _w((lambda *s: _rng.normal(s) * 0.05)(1, 576) * 8.0), 'w_mod': _w((lambda *s: _rng.normal(s) * 0.05)(576, 6 * 576) * 576 ** (-0.5) * 8.0)}

def reference(A_x, A_wqkv, A_wo, B_x, B_w1, B_w2, c, w_mod):

    def _A_ref(x, wqkv, wo):
        B, S, D = x.shape
        H = 32
        Dh = D // H
        W, dil = (8, 2)
        qkv = (lambda x, *d: x.transpose(*d))((x @ wqkv).reshape(B, S, 3, H, Dh), 2, 0, 3, 1, 4)
        q, k, v = (qkv[0], qkv[1], qkv[2])
        scale = Dh ** (-0.5)
        pos = jnp.arange(S)
        off = jnp.arange(W) * dil
        idx = pos[:, None] - off[None, :]
        mask = idx >= 0
        idx_c = jnp.where(mask, idx, 0).reshape(-1)
        kg = k[:, :, idx_c, :].reshape(B, H, S, W, Dh)
        vg = v[:, :, idx_c, :].reshape(B, H, S, W, Dh)
        logits = jnp.einsum('bhsd,bhswd->bhsw', q, kg) * scale
        logits = jnp.where(mask[None, None, :, :], logits, -1000000000.0)
        attn = _softmax(logits, axis=-1)
        o = jnp.einsum('bhsw,bhswd->bhsd', attn, vg)
        return (lambda x, *d: x.transpose(*d))(o, 0, 2, 1, 3).reshape(B, S, D) @ wo

    def _B_ref(x, w1, w2):
        h = jnp.einsum('bsd,df->bsf', x, w1)
        zero = jnp.zeros_like(h)
        h = jnp.maximum(h, zero)
        return jnp.einsum('bsf,fd->bsd', h, w2)
    x = A_x
    mod = (_silu(c) @ w_mod).reshape(c.shape[0], 6, 1, -1)
    sa, ca, ga, sb, cb, gb = (mod[:, 0].copy(), mod[:, 1].copy(), mod[:, 2].copy(), mod[:, 3].copy(), mod[:, 4].copy(), mod[:, 5].copy())
    h = _layernorm(x, axis=-1) * (1 + ca) + sa
    x = x + ga * _A_ref(h, A_wqkv, A_wo)
    h = _layernorm(x, axis=-1) * (1 + cb) + sb
    x = x + gb * _B_ref(h, B_w1, B_w2)
    return x
```

```python
import functools

import jax
import jax.numpy as jnp
import jax.experimental.pallas as pl
import jax.experimental.pallas.tpu as pltpu

S = 2048
D = 576
H = 32
DH = D // H
W = 8
DIL = 2
DFF = 4608
DP = 640
HALO = 16
T = 512
FC = 512
NFC = DFF // FC
RC = 32
EPS = 1e-5
SCALE = DH ** (-0.5)
NEG = -1000000000.0

_bf16 = jnp.bfloat16
_f32 = jnp.float32


def _ln_mod(x, scale_row, shift_row):
    m = jnp.mean(x, axis=-1, keepdims=True)
    xc = x - m
    v = jnp.mean(xc * xc, axis=-1, keepdims=True)
    return xc * jax.lax.rsqrt(v + EPS) * scale_row + shift_row


def _kernel(c_ref, x_ref, wqkv_hbm, wo_hbm, w1_hbm, w2_hbm, wmod_hbm,
            o_ref,
            wqkv_raw, wqkv_p, wo_raw, wo_p, w1_v, w2_v, wmod_v, mod_v,
            kbuf, vbuf, obuf, sems):
    i = pl.program_id(0)

    SEM_WQKV, SEM_WMODA, SEM_WO, SEM_WMODB = 0, 1, 2, 3
    SEM_W1, SEM_W2 = 4, 4 + NFC

    def cp_wqkv():
        return pltpu.make_async_copy(wqkv_hbm, wqkv_raw, sems.at[SEM_WQKV])

    def cp_wmoda():
        return pltpu.make_async_copy(wmod_hbm.at[:, pl.ds(0, 2 * D)],
                                     wmod_v.at[:, pl.ds(0, 2 * D)], sems.at[SEM_WMODA])

    def cp_wmodb():
        return pltpu.make_async_copy(wmod_hbm.at[:, pl.ds(2 * D, 4 * D)],
                                     wmod_v.at[:, pl.ds(2 * D, 4 * D)], sems.at[SEM_WMODB])

    def cp_wo():
        return pltpu.make_async_copy(wo_hbm, wo_raw, sems.at[SEM_WO])

    def cp_w1(j):
        return pltpu.make_async_copy(w1_hbm.at[:, pl.ds(j * FC, FC)],
                                     w1_v.at[:, pl.ds(j * FC, FC)], sems.at[SEM_W1 + j])

    def cp_w2(j):
        return pltpu.make_async_copy(w2_hbm.at[pl.ds(j * FC, FC), :],
                                     w2_v.at[pl.ds(j * FC, FC), :], sems.at[SEM_W2 + j])

    @pl.when(i == 0)
    def _prologue():
        cp_wqkv().start()
        cp_wmoda().start()
        cp_wo().start()
        cp_wmodb().start()
        for j in range(NFC):
            cp_w1(j).start()
            cp_w2(j).start()

        kbuf[0:HALO, :] = jnp.zeros((HALO, DP), _f32)
        vbuf[0:HALO, :] = jnp.zeros((HALO, DP), _f32)

        r = jax.lax.broadcasted_iota(jnp.int32, (D, DP), 0)
        cidx = jax.lax.broadcasted_iota(jnp.int32, (D, DP), 1)
        hh = cidx & (H - 1)
        dd = cidx >> 5
        pmat = jnp.where((r == hh * DH + dd) & (dd < DH), 1.0, 0.0).astype(_bf16)

        cp_wqkv().wait()
        for j in range(3):
            wqkv_p[:, j * DP:(j + 1) * DP] = jnp.dot(
                wqkv_raw[:, j * D:(j + 1) * D], pmat,
                preferred_element_type=_f32).astype(_bf16)

        cp_wmoda().wait()
        c = c_ref[...].astype(_f32)
        sc = (c * jax.nn.sigmoid(c)).astype(_bf16)
        sc8 = jnp.broadcast_to(sc, (8, D))
        mod_v[:, 0:2 * D] = jnp.dot(sc8, wmod_v[:, 0:2 * D], preferred_element_type=_f32)

    x = x_ref[...].astype(_f32)
    sa = mod_v[0:1, 0:D]
    ca = mod_v[0:1, D:2 * D]
    h = _ln_mod(x, 1.0 + ca, sa).astype(_bf16)

    qkv = jnp.dot(h, wqkv_p[...], preferred_element_type=_f32)
    obuf[...] = qkv[:, 0:DP] * SCALE
    kbuf[HALO:HALO + T, :] = qkv[:, DP:2 * DP]
    vbuf[HALO:HALO + T, :] = qkv[:, 2 * DP:3 * DP]

    def attn_chunk(rc, carry):
        r0 = pl.multiple_of(rc * RC, RC)
        q = obuf[pl.ds(r0, RC), :]
        pos = i * T + r0 + jax.lax.broadcasted_iota(jnp.int32, (RC, 128), 0)
        kwin = kbuf[pl.ds(r0, RC + HALO), :]
        vwin = vbuf[pl.ds(r0, RC + HALO), :]
        logits = []
        for w in range(W):
            kw = kwin[HALO - DIL * w:HALO - DIL * w + RC, :]
            p = q * kw
            s = (p[:, 0:128] + p[:, 128:256]) + (p[:, 256:384] + p[:, 384:512]) + p[:, 512:640]
            s = s + pltpu.roll(s, 64, 1)
            s = s + pltpu.roll(s, 32, 1)
            if w > 0:
                s = jnp.where(pos >= DIL * w, s, NEG)
            logits.append(s)
        m = logits[0]
        for w in range(1, W):
            m = jnp.maximum(m, logits[w])
        es = [jnp.exp(l - m) for l in logits]
        den = es[0]
        for w in range(1, W):
            den = den + es[w]
        inv = 1.0 / den
        acc = None
        for w in range(W):
            vw = vwin[HALO - DIL * w:HALO - DIL * w + RC, :]
            a = es[w] * inv
            a5 = jnp.concatenate([a] * 5, axis=1)
            acc = a5 * vw if acc is None else acc + a5 * vw
        obuf[pl.ds(r0, RC), :] = acc
        return carry

    jax.lax.fori_loop(0, T // RC, attn_chunk, 0)

    kbuf[0:HALO, :] = kbuf[T:T + HALO, :]
    vbuf[0:HALO, :] = vbuf[T:T + HALO, :]

    @pl.when(i == 0)
    def _prologue2():
        cp_wo().wait()
        r = jax.lax.broadcasted_iota(jnp.int32, (DP, D), 0)
        cidx = jax.lax.broadcasted_iota(jnp.int32, (DP, D), 1)
        hh = r & (H - 1)
        dd = r >> 5
        pmat_t = jnp.where((cidx == hh * DH + dd) & (dd < DH), 1.0, 0.0).astype(_bf16)
        wo_p[...] = jnp.dot(pmat_t, wo_raw[...], preferred_element_type=_f32).astype(_bf16)
        cp_wmodb().wait()
        c = c_ref[...].astype(_f32)
        sc = (c * jax.nn.sigmoid(c)).astype(_bf16)
        sc8 = jnp.broadcast_to(sc, (8, D))
        mod_v[:, 2 * D:6 * D] = jnp.dot(sc8, wmod_v[:, 2 * D:6 * D], preferred_element_type=_f32)

    ga = mod_v[0:1, 2 * D:3 * D]
    sb = mod_v[0:1, 3 * D:4 * D]
    cb = mod_v[0:1, 4 * D:5 * D]
    gb = mod_v[0:1, 5 * D:6 * D]

    attn = jnp.dot(obuf[...].astype(_bf16), wo_p[...], preferred_element_type=_f32)
    x1 = x + ga * attn
    h2 = _ln_mod(x1, 1.0 + cb, sb).astype(_bf16)

    acc = None
    for j in range(NFC):
        @pl.when(i == 0)
        def _wait_chunk():
            cp_w1(j).wait()
            cp_w2(j).wait()
        h1 = jnp.dot(h2, w1_v[:, j * FC:(j + 1) * FC], preferred_element_type=_f32)
        h1 = jnp.maximum(h1, 0.0).astype(_bf16)
        part = jnp.dot(h1, w2_v[j * FC:(j + 1) * FC, :], preferred_element_type=_f32)
        acc = part if acc is None else acc + part

    o_ref[...] = (x1 + gb * acc).astype(o_ref.dtype)


@jax.jit
def pallas_adaLN_cond__sliding_local_dilated__dense_activation_relu__prompt_kernel(
    A_x: jax.Array,
    A_wqkv: jax.Array,
    A_wo: jax.Array,
    B_x: jax.Array,
    B_w1: jax.Array,
    B_w2: jax.Array,
    c: jax.Array,
    w_mod: jax.Array,
):
    del B_x
    x2d = A_x.reshape(S, D)
    any_spec = pl.BlockSpec(memory_space=pl.ANY)
    out = pl.pallas_call(
        _kernel,
        grid=(S // T,),
        in_specs=[
            pl.BlockSpec((1, D), lambda i: (0, 0)),
            pl.BlockSpec((T, D), lambda i: (i, 0)),
            any_spec, any_spec, any_spec, any_spec, any_spec,
        ],
        out_specs=pl.BlockSpec((T, D), lambda i: (i, 0)),
        out_shape=jax.ShapeDtypeStruct((S, D), _bf16),
        scratch_shapes=[
            pltpu.VMEM((D, 3 * D), _bf16),
            pltpu.VMEM((D, 3 * DP), _bf16),
            pltpu.VMEM((D, D), _bf16),
            pltpu.VMEM((DP, D), _bf16),
            pltpu.VMEM((D, DFF), _bf16),
            pltpu.VMEM((DFF, D), _bf16),
            pltpu.VMEM((D, 6 * D), _bf16),
            pltpu.VMEM((8, 6 * D), _f32),
            pltpu.VMEM((T + HALO, DP), _f32),
            pltpu.VMEM((T + HALO, DP), _f32),
            pltpu.VMEM((T, DP), _f32),
            pltpu.SemaphoreType.DMA((4 + 2 * NFC,)),
        ],
        compiler_params=pltpu.CompilerParams(
            dimension_semantics=("arbitrary",),
            vmem_limit_bytes=100 * 1024 * 1024,
        ),
    )(c, x2d, A_wqkv, A_wo, B_w1, B_w2, w_mod)
    return out.reshape(1, S, D)
```

```python
import contextlib

import jax
import jax.numpy as jnp
import jax.experimental.pallas as pl
import jax.experimental.pallas.tpu as pltpu

S = 2048
D = 576
H = 32
DH = D // H
W = 8
DIL = 2
DFF = 4608
LANES = 128
HB = 16
T = 512
NTILES = S // T
FC = 512
NFC = DFF // FC
EPS = 1e-5
SCALE = DH ** (-0.5)
NEG = -1000000000.0

_PROFILE_SCOPES = False


def _scope(name):
    return jax.named_scope(name) if _PROFILE_SCOPES else contextlib.nullcontext()


_bf16 = jnp.bfloat16
_f32 = jnp.float32
_NT = (((1,), (1,)), ((), ()))


def _ln_mod_t(x, scale_col, shift_col):
    m = jnp.mean(x, axis=0, keepdims=True)
    xc = x - m
    v = jnp.mean(xc * xc, axis=0, keepdims=True)
    xn = xc * jax.lax.rsqrt(v + EPS)
    reps = x.shape[1] // LANES
    sc = jnp.concatenate([scale_col] * reps, axis=1)
    sh = jnp.concatenate([shift_col] * reps, axis=1)
    return xn * sc + sh


def _kernel(c_ref, x_ref, wqkv_hbm, wo_hbm, w1_hbm, w2t_hbm, wmod_hbm,
            o_ref,
            wqkv_raw, wqkvt_p, wo_raw, wot_p, w1_raw, w1t, w2t_v, wmod_v, modc,
            kbuf, vbuf, ksh, vsh, obuf, h2buf, x1buf, accbuf, tbuf, sems):
    i = pl.program_id(0)

    SEM_WQKV, SEM_WMODA, SEM_WO, SEM_WMODB = 0, 1, 2, 3
    SEM_W1, SEM_W2 = 4, 4 + NFC

    def cp_wqkv():
        return pltpu.make_async_copy(wqkv_hbm, wqkv_raw, sems.at[SEM_WQKV])

    def cp_wmoda():
        return pltpu.make_async_copy(wmod_hbm.at[:, pl.ds(0, 2 * D)],
                                     wmod_v.at[:, pl.ds(0, 2 * D)], sems.at[SEM_WMODA])

    def cp_wmodb():
        return pltpu.make_async_copy(wmod_hbm.at[:, pl.ds(2 * D, 4 * D)],
                                     wmod_v.at[:, pl.ds(2 * D, 4 * D)], sems.at[SEM_WMODB])

    def cp_wo():
        return pltpu.make_async_copy(wo_hbm, wo_raw, sems.at[SEM_WO])

    def cp_w1(j):
        return pltpu.make_async_copy(w1_hbm.at[:, pl.ds(j * FC, FC)],
                                     w1_raw.at[:, pl.ds(j * FC, FC)], sems.at[SEM_W1 + j])

    def cp_w2(j):
        return pltpu.make_async_copy(w2t_hbm.at[:, pl.ds(j * FC, FC)],
                                     w2t_v.at[:, pl.ds(j * FC, FC)], sems.at[SEM_W2 + j])

    def perm_t():
        cc = jax.lax.broadcasted_iota(jnp.int32, (D, D), 0)
        rr = jax.lax.broadcasted_iota(jnp.int32, (D, D), 1)
        return jnp.where(rr == (cc & (H - 1)) * DH + (cc >> 5), 1.0, 0.0).astype(_bf16)

    NCB = (D + LANES - 1) // LANES

    def stage(val):
        for cb in range(NCB):
            w = min(LANES, D - cb * LANES)
            tbuf[cb, :, 0:w] = val[:, cb * LANES:cb * LANES + w]

    def perm_rows(d):
        parts = [tbuf[cb, pl.ds(d, H, stride=DH), :] for cb in range(NCB)]
        parts[-1] = parts[-1][:, 0:D - (NCB - 1) * LANES]
        return jnp.concatenate(parts, axis=1)

    def mod_cols(first, count):
        c = c_ref[...].astype(_f32)
        sc = (c * jax.nn.sigmoid(c)).astype(_bf16)
        sc8 = jnp.broadcast_to(sc, (8, D))
        for s in range(first, first + count):
            row = jnp.dot(sc8, wmod_v[:, s * D:(s + 1) * D], preferred_element_type=_f32)
            col = row.T
            modc[s] = jnp.broadcast_to(col[:, 0:1], (D, LANES))

    NT = pl.num_programs(0) - 1
    reps = T // LANES
    NCH = T // LANES

    def bcast(col):
        return jnp.concatenate([col] * reps, axis=1)

    def prologue():
        cp_wqkv().start()
        cp_wmoda().start()
        kbuf[:, 0:LANES] = jnp.zeros((D, LANES), _bf16)
        vbuf[:, 0:LANES] = jnp.zeros((D, LANES), _bf16)
        cp_wqkv().wait()
        cp_wo().start()
        cp_wmodb().start()
        for j in range(NFC):
            cp_w1(j).start()
        for j in range(NFC):
            cp_w2(j).start()
        tbuf[NCB - 1] = jnp.zeros((D, LANES), _f32)
        for j in range(3):
            stage(wqkv_raw[:, j * D:(j + 1) * D].astype(_f32).T)
            for d in range(DH):
                wqkvt_p[j * D + d * H:j * D + (d + 1) * H, :] = perm_rows(d).astype(_bf16)
        cp_wmoda().wait()
        mod_cols(0, 2)

    def prologue2():
        cp_wo().wait()
        stage(wo_raw[...].astype(_f32))
        wo_p = jnp.concatenate([perm_rows(d) for d in range(DH)], axis=0)
        wot_p[...] = wo_p.T.astype(_bf16)
        cp_wmodb().wait()
        mod_cols(2, 4)

    def prologue3():
        def body(j, carry):
            f0 = pl.multiple_of(j * FC, FC)
            cp_w1(j).wait()
            w1t[pl.ds(f0, FC), :] = (
                w1_raw[:, pl.ds(f0, FC)].astype(_f32).T.astype(_bf16))
            cp_w2(j).wait()
            return carry
        jax.lax.fori_loop(0, NFC, body, 0)

    def a_front():
        x = x_ref[...].astype(_f32)
        h = _ln_mod_t(x, 1.0 + modc[1], modc[0]).astype(_bf16)
        qkv = jnp.dot(wqkvt_p[...], h, preferred_element_type=_f32)
        obuf[...] = qkv[0:D, :] * SCALE
        kbuf[:, LANES:LANES + T] = qkv[D:2 * D, :].astype(_bf16)
        vbuf[:, LANES:LANES + T] = qkv[2 * D:3 * D, :].astype(_bf16)

    def shift(w):
        for src, dst in ((kbuf, ksh), (vbuf, vsh)):
            full = pltpu.bitcast(src[...], jnp.uint32)
            rolled = pltpu.roll(full, DIL * w, 1)
            dst[w - 1] = pltpu.bitcast(rolled[:, LANES:], _bf16)

    def attn_chunk(j):
        l0 = pl.multiple_of(j * LANES, LANES)
        pos = i * T + l0 + jax.lax.broadcasted_iota(jnp.int32, (HB, LANES), 1)
        for hb in range(H // HB):
            logits = [None] * W
            for d in range(DH):
                rows = slice(d * H + hb * HB, d * H + (hb + 1) * HB)
                q = obuf[rows, pl.ds(l0, LANES)]
                for w in range(W):
                    if w == 0:
                        kw = kbuf[rows, pl.ds(l0 + LANES, LANES)]
                    else:
                        kw = ksh[w - 1, rows, pl.ds(l0, LANES)]
                    p = q * kw.astype(_f32)
                    logits[w] = p if logits[w] is None else logits[w] + p
            for w in range(1, W):
                logits[w] = jnp.where(pos >= DIL * w, logits[w], NEG)
            m = logits[0]
            for w in range(1, W):
                m = jnp.maximum(m, logits[w])
            es = [jnp.exp(l - m) for l in logits]
            den = es[0]
            for w in range(1, W):
                den = den + es[w]
            inv = 1.0 / den
            ps = [e * inv for e in es]
            for d in range(DH):
                rows = slice(d * H + hb * HB, d * H + (hb + 1) * HB)
                acc = None
                for w in range(W):
                    if w == 0:
                        vw = vbuf[rows, pl.ds(l0 + LANES, LANES)]
                    else:
                        vw = vsh[w - 1, rows, pl.ds(l0, LANES)]
                    t = ps[w] * vw.astype(_f32)
                    acc = t if acc is None else acc + t
                obuf[rows, pl.ds(l0, LANES)] = acc

    def a_back():
        kbuf[:, 0:LANES] = kbuf[:, T:T + LANES]
        vbuf[:, 0:LANES] = vbuf[:, T:T + LANES]
        attn = jnp.dot(wot_p[...], obuf[...].astype(_bf16), preferred_element_type=_f32)
        x1 = x_ref[...].astype(_f32) + bcast(modc[2]) * attn
        x1buf[...] = x1
        h2buf[...] = _ln_mod_t(x1, 1.0 + modc[4], modc[3]).astype(_bf16)

    def mlp_chunk(j):
        f0 = pl.multiple_of(j * FC, FC)
        h1 = jnp.dot(w1t[pl.ds(f0, FC), :], h2buf[...], preferred_element_type=_f32)
        h1 = jnp.maximum(h1, 0.0).astype(_bf16)
        accbuf[...] += jnp.dot(w2t_v[:, pl.ds(f0, FC)], h1, preferred_element_type=_f32)

    def m_final():
        o_ref[...] = (x1buf[...] + bcast(modc[5]) * accbuf[...]).astype(o_ref.dtype)

    CPI = NCH // 2

    def run(do_a, do_m):
        if do_m:
            accbuf[...] = jnp.zeros((D, T), _f32)
        if do_a:
            with _scope("a_front"):
                a_front()

        def body1(j, carry):
            if do_m:
                mlp_chunk(j)
            if do_a:
                shift(j + 1)
            return carry

        def body2(j, carry):
            if do_m:
                mlp_chunk(j)
            if do_a:
                for u in range(CPI):
                    attn_chunk((j - (W - 1)) * CPI + u)
            return carry

        with _scope("loop1"):
            jax.lax.fori_loop(0, W - 1, body1, 0)
        with _scope("loop2"):
            jax.lax.fori_loop(W - 1, NFC, body2, 0)
        if do_m:
            with _scope("m_final"):
                m_final()

    @pl.when(i == 0)
    def _first():
        with _scope("prologue"):
            prologue()
        run(True, False)
        with _scope("prologue2"):
            prologue2()
        with _scope("a_back"):
            a_back()
        with _scope("prologue3"):
            prologue3()

    @pl.when(jnp.logical_and(i > 0, i < NT))
    def _mid():
        run(True, True)
        with _scope("a_back"):
            a_back()

    @pl.when(i == NT)
    def _last():
        run(False, True)


@jax.jit
def pallas_adaLN_cond__sliding_local_dilated__dense_activation_relu__prompt_kernel(
    A_x: jax.Array,
    A_wqkv: jax.Array,
    A_wo: jax.Array,
    B_x: jax.Array,
    B_w1: jax.Array,
    B_w2: jax.Array,
    c: jax.Array,
    w_mod: jax.Array,
):
    del B_x
    xt = A_x.reshape(S, D).T
    w2t = B_w2.T
    hbm_spec = pl.BlockSpec(memory_space=pltpu.MemorySpace.HBM)
    out_t = pl.pallas_call(
        _kernel,
        grid=(NTILES + 1,),
        in_specs=[
            pl.BlockSpec((1, D), lambda i: (0, 0)),
            pl.BlockSpec((D, T), lambda i: (0, jnp.minimum(i, NTILES - 1))),
            hbm_spec, hbm_spec, hbm_spec, hbm_spec, hbm_spec,
        ],
        out_specs=pl.BlockSpec((D, T), lambda i: (0, jnp.maximum(i - 1, 0))),
        out_shape=jax.ShapeDtypeStruct((D, S), _bf16),
        scratch_shapes=[
            pltpu.VMEM((D, 3 * D), _bf16),
            pltpu.VMEM((3 * D, D), _bf16),
            pltpu.VMEM((D, D), _bf16),
            pltpu.VMEM((D, D), _bf16),
            pltpu.VMEM((D, DFF), _bf16),
            pltpu.VMEM((DFF, D), _bf16),
            pltpu.VMEM((D, DFF), _bf16),
            pltpu.VMEM((D, 6 * D), _bf16),
            pltpu.VMEM((6, D, LANES), _f32),
            pltpu.VMEM((D, T + LANES), _bf16),
            pltpu.VMEM((D, T + LANES), _bf16),
            pltpu.VMEM((W - 1, D, T), _bf16),
            pltpu.VMEM((W - 1, D, T), _bf16),
            pltpu.VMEM((D, T), _f32),
            pltpu.VMEM((D, T), _bf16),
            pltpu.VMEM((D, T), _f32),
            pltpu.VMEM((D, T), _f32),
            pltpu.VMEM((5, D, LANES), _f32),
            pltpu.SemaphoreType.DMA((4 + 2 * NFC,)),
        ],
        compiler_params=pltpu.CompilerParams(
            dimension_semantics=("arbitrary",),
            vmem_limit_bytes=100 * 1024 * 1024,
        ),
    )(c, xt, A_wqkv, A_wo, B_w1, w2t, w_mod)
    return out_t.T.reshape(1, S, D)
```

```python
import contextlib

import jax
import jax.numpy as jnp
import jax.experimental.pallas as pl
import jax.experimental.pallas.tpu as pltpu

S = 2048
D = 576
H = 32
DH = D // H
W = 8
DIL = 2
DFF = 4608
LANES = 128
NSUB = 2
HB = 16
T = 512
NTILES = S // T
TS = T // NSUB
FC = 512
NFC = DFF // FC
EPS = 1e-5
SCALE = DH ** (-0.5)
NEG = -1000000000.0

_PROFILE_SCOPES = False


def _scope(name):
    return jax.named_scope(name) if _PROFILE_SCOPES else contextlib.nullcontext()


_bf16 = jnp.bfloat16
_f32 = jnp.float32
_NT = (((1,), (1,)), ((), ()))


def _ln_mod_t(x, scale_col, shift_col):
    m = jnp.mean(x, axis=0, keepdims=True)
    xc = x - m
    v = jnp.mean(xc * xc, axis=0, keepdims=True)
    xn = xc * jax.lax.rsqrt(v + EPS)
    reps = x.shape[1] // LANES
    sc = jnp.concatenate([scale_col] * reps, axis=1)
    sh = jnp.concatenate([shift_col] * reps, axis=1)
    return xn * sc + sh


def _kernel(c_ref, x_ref, wqkv_hbm, wo_hbm, w1_hbm, w2t_hbm, wmod_hbm,
            o_ref,
            wqkv_raw, wqkvt_p, wo_raw, wot_p, w1_raw, w1t, w2t_v, wmod_v, modc,
            kbuf, vbuf, ksh, vsh, obuf, h2buf, x1buf, accbuf, tbuf, sems):
    i = pl.program_id(0)

    SEM_WQKV, SEM_WMODA, SEM_WO, SEM_WMODB = 0, 1, 2, 3
    SEM_W1, SEM_W2 = 4, 4 + NFC

    def cp_wqkv():
        return pltpu.make_async_copy(wqkv_hbm, wqkv_raw, sems.at[SEM_WQKV])

    def cp_wmoda():
        return pltpu.make_async_copy(wmod_hbm.at[:, pl.ds(0, 2 * D)],
                                     wmod_v.at[:, pl.ds(0, 2 * D)], sems.at[SEM_WMODA])

    def cp_wmodb():
        return pltpu.make_async_copy(wmod_hbm.at[:, pl.ds(2 * D, 4 * D)],
                                     wmod_v.at[:, pl.ds(2 * D, 4 * D)], sems.at[SEM_WMODB])

    def cp_wo():
        return pltpu.make_async_copy(wo_hbm, wo_raw, sems.at[SEM_WO])

    def cp_w1(j):
        return pltpu.make_async_copy(w1_hbm.at[:, pl.ds(j * FC, FC)],
                                     w1_raw.at[:, pl.ds(j * FC, FC)], sems.at[SEM_W1 + j])

    def cp_w2(j):
        return pltpu.make_async_copy(w2t_hbm.at[:, pl.ds(j * FC, FC)],
                                     w2t_v.at[:, pl.ds(j * FC, FC)], sems.at[SEM_W2 + j])

    NCB = (D + LANES - 1) // LANES

    def stage(val):
        for cb in range(NCB):
            w = min(LANES, D - cb * LANES)
            tbuf[cb, :, 0:w] = val[:, cb * LANES:cb * LANES + w]

    def perm_rows(d):
        parts = [tbuf[cb, pl.ds(d, H, stride=DH), :] for cb in range(NCB)]
        parts[-1] = parts[-1][:, 0:D - (NCB - 1) * LANES]
        return jnp.concatenate(parts, axis=1)

    def mod_cols(first, count):
        c = c_ref[...].astype(_f32)
        sc = (c * jax.nn.sigmoid(c)).astype(_bf16)
        sc8 = jnp.broadcast_to(sc, (8, D))
        for s in range(first, first + count):
            row = jnp.dot(sc8, wmod_v[:, s * D:(s + 1) * D], preferred_element_type=_f32)
            col = row.T
            modc[s] = jnp.broadcast_to(col[:, 0:1], (D, LANES))

    NT = pl.num_programs(0) - 1
    reps = T // LANES
    NCH = T // LANES

    def bcast(col):
        return jnp.concatenate([col] * reps, axis=1)

    def prologue():
        cp_wqkv().start()
        cp_wmoda().start()
        kbuf[:, 0:LANES] = jnp.zeros((D, LANES), _bf16)
        vbuf[:, 0:LANES] = jnp.zeros((D, LANES), _bf16)
        cp_wqkv().wait()
        for j in range(NFC):
            cp_w1(j).start()
        cp_wo().start()
        cp_wmodb().start()
        for j in range(NFC):
            cp_w2(j).start()
        tbuf[NCB - 1] = jnp.zeros((D, LANES), _f32)
        for j in range(3):
            stage(wqkv_raw[:, j * D:(j + 1) * D].astype(_f32).T)
            for d in range(DH):
                wqkvt_p[j * D + d * H:j * D + (d + 1) * H, :] = perm_rows(d).astype(_bf16)
        cp_wmoda().wait()
        mod_cols(0, 2)

    def prologue2():
        cp_wo().wait()
        stage(wo_raw[...].astype(_f32))
        wo_p = jnp.concatenate([perm_rows(d) for d in range(DH)], axis=0)
        wot_p[...] = wo_p.T.astype(_bf16)
        cp_wmodb().wait()
        mod_cols(2, 4)

    def prep_w1(j):
        f0 = pl.multiple_of(j * FC, FC)
        rr = jax.lax.broadcasted_iota(jnp.int32, (LANES, LANES), 0)
        cc = jax.lax.broadcasted_iota(jnp.int32, (LANES, LANES), 1)
        eye = jnp.where(rr == cc, 1.0, 0.0).astype(_bf16)
        cp_w1(j).wait()
        for u in range(FC // LANES):
            c0 = pl.multiple_of(f0 + u * LANES, LANES)
            w1t[pl.ds(c0, LANES), :] = jax.lax.dot_general(
                eye, w1_raw[:, pl.ds(c0, LANES)], _NT,
                preferred_element_type=_f32).astype(_bf16)

    def wait_w2():
        for j in range(NFC):
            cp_w2(j).wait()

    def shifts(src, dst):
        full = pltpu.bitcast(src[...], jnp.uint32)
        for w in range(1, W):
            rolled = pltpu.roll(full, DIL * w, 1)
            dst[w - 1] = pltpu.bitcast(rolled[:, LANES:], _bf16)

    def a_front():
        x = x_ref[...].astype(_f32)
        h = _ln_mod_t(x, 1.0 + modc[1], modc[0]).astype(_bf16)
        kbuf[:, LANES:LANES + T] = jnp.dot(
            wqkvt_p[D:2 * D, :], h, preferred_element_type=_f32).astype(_bf16)
        vbuf[:, LANES:LANES + T] = jnp.dot(
            wqkvt_p[2 * D:3 * D, :], h, preferred_element_type=_f32).astype(_bf16)
        shifts(kbuf, ksh)
        obuf[...] = SCALE * jnp.dot(wqkvt_p[0:D, :], h, preferred_element_type=_f32)
        shifts(vbuf, vsh)

    def attn_chunk(j):
        l0 = pl.multiple_of(j * LANES, LANES)
        pos = i * T + l0 + jax.lax.broadcasted_iota(jnp.int32, (HB, LANES), 1)
        for hb in range(H // HB):
            logits = [None] * W
            for d in range(DH):
                rows = slice(d * H + hb * HB, d * H + (hb + 1) * HB)
                q = obuf[rows, pl.ds(l0, LANES)]
                for w in range(W):
                    if w == 0:
                        kw = kbuf[rows, pl.ds(l0 + LANES, LANES)]
                    else:
                        kw = ksh[w - 1, rows, pl.ds(l0, LANES)]
                    p = q * kw.astype(_f32)
                    logits[w] = p if logits[w] is None else logits[w] + p
            for w in range(1, W):
                logits[w] = jnp.where(pos >= DIL * w, logits[w], NEG)
            m = logits[0]
            for w in range(1, W):
                m = jnp.maximum(m, logits[w])
            es = [jnp.exp(l - m) for l in logits]
            den = es[0]
            for w in range(1, W):
                den = den + es[w]
            inv = 1.0 / den
            ps = [e * inv for e in es]
            for d in range(DH):
                rows = slice(d * H + hb * HB, d * H + (hb + 1) * HB)
                acc = None
                for w in range(W):
                    if w == 0:
                        vw = vbuf[rows, pl.ds(l0 + LANES, LANES)]
                    else:
                        vw = vsh[w - 1, rows, pl.ds(l0, LANES)]
                    t = ps[w] * vw.astype(_f32)
                    acc = t if acc is None else acc + t
                obuf[rows, pl.ds(l0, LANES)] = acc

    def a_back():
        kbuf[:, 0:LANES] = kbuf[:, T:T + LANES]
        vbuf[:, 0:LANES] = vbuf[:, T:T + LANES]
        for u in range(NSUB):
            cols = slice(u * TS, (u + 1) * TS)
            attn = jnp.dot(wot_p[...], obuf[:, cols].astype(_bf16),
                           preferred_element_type=_f32)
            ga = jnp.concatenate([modc[2]] * (TS // LANES), axis=1)
            x1 = x_ref[:, cols].astype(_f32) + ga * attn
            x1buf[:, cols] = x1
            h2buf[:, cols] = _ln_mod_t(x1, 1.0 + modc[4], modc[3]).astype(_bf16)

    def mlp_chunk(j):
        f0 = pl.multiple_of(j * FC, FC)
        h1 = jnp.dot(w1t[pl.ds(f0, FC), :], h2buf[...], preferred_element_type=_f32)
        h1 = jnp.maximum(h1, 0.0).astype(_bf16)
        accbuf[...] += jnp.dot(w2t_v[:, pl.ds(f0, FC)], h1, preferred_element_type=_f32)

    def m_final():
        o_ref[...] = (x1buf[...] + bcast(modc[5]) * accbuf[...]).astype(o_ref.dtype)

    CPI = NCH // 2

    def run(do_a, do_m):
        if do_m:
            accbuf[...] = jnp.zeros((D, T), _f32)
        if do_a:
            with _scope("a_front"):
                a_front()

        def body1(j, carry):
            if do_m:
                mlp_chunk(j)
            else:
                prep_w1(j)
            return carry

        def body2(j, carry):
            if do_m:
                mlp_chunk(j)
            else:
                prep_w1(j)
            if do_a:
                for u in range(CPI):
                    attn_chunk((j - (W - 1)) * CPI + u)
            return carry

        with _scope("loop1"):
            jax.lax.fori_loop(0, W - 1, body1, 0)
        with _scope("loop2"):
            jax.lax.fori_loop(W - 1, NFC, body2, 0)
        if do_m:
            with _scope("m_final"):
                m_final()

    @pl.when(i == 0)
    def _first():
        with _scope("prologue"):
            prologue()
        run(True, False)
        with _scope("prologue2"):
            prologue2()
        with _scope("a_back"):
            a_back()
        wait_w2()

    @pl.when(jnp.logical_and(i > 0, i < NT))
    def _mid():
        run(True, True)
        with _scope("a_back"):
            a_back()

    @pl.when(i == NT)
    def _last():
        run(False, True)


@jax.jit
def pallas_adaLN_cond__sliding_local_dilated__dense_activation_relu__prompt_kernel(
    A_x: jax.Array,
    A_wqkv: jax.Array,
    A_wo: jax.Array,
    B_x: jax.Array,
    B_w1: jax.Array,
    B_w2: jax.Array,
    c: jax.Array,
    w_mod: jax.Array,
):
    del B_x
    xt = A_x.reshape(S, D).T
    w2t = B_w2.T
    hbm_spec = pl.BlockSpec(memory_space=pltpu.MemorySpace.HBM)
    out_t = pl.pallas_call(
        _kernel,
        grid=(NTILES + 1,),
        in_specs=[
            pl.BlockSpec((1, D), lambda i: (0, 0)),
            pl.BlockSpec((D, T), lambda i: (0, jnp.minimum(i, NTILES - 1))),
            hbm_spec, hbm_spec, hbm_spec, hbm_spec, hbm_spec,
        ],
        out_specs=pl.BlockSpec((D, T), lambda i: (0, jnp.maximum(i - 1, 0))),
        out_shape=jax.ShapeDtypeStruct((D, S), _bf16),
        scratch_shapes=[
            pltpu.VMEM((D, 3 * D), _bf16),
            pltpu.VMEM((3 * D, D), _bf16),
            pltpu.VMEM((D, D), _bf16),
            pltpu.VMEM((D, D), _bf16),
            pltpu.VMEM((D, DFF), _bf16),
            pltpu.VMEM((DFF, D), _bf16),
            pltpu.VMEM((D, DFF), _bf16),
            pltpu.VMEM((D, 6 * D), _bf16),
            pltpu.VMEM((6, D, LANES), _f32),
            pltpu.VMEM((D, T + LANES), _bf16),
            pltpu.VMEM((D, T + LANES), _bf16),
            pltpu.VMEM((W - 1, D, T), _bf16),
            pltpu.VMEM((W - 1, D, T), _bf16),
            pltpu.VMEM((D, T), _f32),
            pltpu.VMEM((D, T), _bf16),
            pltpu.VMEM((D, T), _f32),
            pltpu.VMEM((D, T), _f32),
            pltpu.VMEM((5, D, LANES), _f32),
            pltpu.SemaphoreType.DMA((4 + 2 * NFC,)),
        ],
        compiler_params=pltpu.CompilerParams(
            dimension_semantics=("arbitrary",),
            vmem_limit_bytes=100 * 1024 * 1024,
        ),
    )(c, xt, A_wqkv, A_wo, B_w1, w2t, w_mod)
    return out_t.T.reshape(1, S, D)
```
